```python
import os as _os
_os.environ.setdefault("JAX_PLATFORMS", "cpu")
import jax
import jax.numpy as jnp

def _softmax(x, axis=-1):
    return jax.nn.softmax(x, axis=axis)
def _gelu(x):
    return jax.nn.gelu(x, approximate=True)
def _silu(x):
    return jax.nn.silu(x)
def _sigmoid(x):
    return jax.nn.sigmoid(x)
def _layernorm(x, axis=-1, eps=1e-5):
    m = jnp.mean(x, axis=axis, keepdims=True)
    v = jnp.var(x, axis=axis, keepdims=True)
    return (x - m) / jnp.sqrt(v + eps)
def _scatter_add(tgt, idx, src, axis=0):
    return tgt.at[idx].add(src)
def _segment_sum(src, seg, n):
    return jax.ops.segment_sum(src, seg, n)
class _Rng:
    def __init__(self, key):
        self._k = key
    def _next(self):
        self._k, sub = jax.random.split(self._k)
        return sub
    def normal(self, shape):
        return jax.random.normal(self._next(), shape, dtype=jnp.bfloat16)
    def randint(self, lo, hi, shape):
        return jax.random.randint(self._next(), shape, lo, hi, dtype=jnp.int32)
    def uniform(self, shape, lo=0.0, hi=1.0):
        return jax.random.uniform(self._next(), shape, jnp.bfloat16, lo, hi)
    def permutation(self, n):
        return jax.random.permutation(self._next(), n)


kernel_name = 'sequential_preLN__softmax_full_mha__swiglu_ffn__prompt'

def setup_inputs():
    _rng = _Rng(jax.random.key(int.from_bytes(__import__("os").urandom(4), "little")))
    _w = (lambda a: (lambda t: t.astype(jnp.bfloat16) if jnp.issubdtype(t.dtype, jnp.floating) else t)(jnp.asarray(a)))
    def _A_setup():
        B, S, D = 1, 2048, 512
        return {
            "x": _w((lambda *s: _rng.normal(s) * 0.05)(B, S, D)),
            "wqkv": _w((lambda *s: _rng.normal(s) * 0.05)(D, 3 * D)),
            "wo": _w((lambda *s: _rng.normal(s) * 0.05)(D, D)),
        }
    _A_in = _A_setup()

    def _B_setup():
        B, S, D, F = 1, 2048, 512, 1792
        return {
            "x": _w((lambda *s: _rng.normal(s) * 0.05)(B, S, D)),
            "w_gate": _w((lambda *s: _rng.normal(s) * 0.05)(D, F)),
            "w_up": _w((lambda *s: _rng.normal(s) * 0.05)(D, F)),
            "w_down": _w((lambda *s: _rng.normal(s) * 0.05)(F, D)),
        }
    _B_in = _B_setup()

    return {
        "A_x": _A_in["x"],
        "A_wqkv": _A_in["wqkv"],
        "A_wo": _A_in["wo"],
        "B_x": _B_in["x"],
        "B_w_gate": _B_in["w_gate"],
        "B_w_up": _B_in["w_up"],
        "B_w_down": _B_in["w_down"],
    }

def reference(A_x, A_wqkv, A_wo, B_x, B_w_gate, B_w_up, B_w_down):
    def _A_ref(x, wqkv, wo):
        B, S, D = x.shape
        H = 32; Dh = D // H
        qkv = (lambda x, *d: x.transpose(*d))((x @ wqkv).reshape(B, S, 3, H, Dh), 2, 0, 3, 1, 4)
        q, k, v = qkv[0], qkv[1], qkv[2]
        scale = Dh ** -0.5
        scores = jnp.einsum("bhqd,bhkd->bhqk", q, k) * scale
        p = _softmax(scores, axis=-1)
        o = jnp.einsum("bhqk,bhkd->bhqd", p, v)
        return (lambda x, *d: x.transpose(*d))(o, 0, 2, 1, 3).reshape(B, S, D) @ wo

    def _B_ref(x, w_gate, w_up, w_down):
        g = _silu(x @ w_gate)
        u = x @ w_up
        return (g * u) @ w_down

    x = A_x
    h = x + _A_ref(_layernorm(x, axis=-1), A_wqkv, A_wo)
    h2 = h + _B_ref(_layernorm(h, axis=-1), B_w_gate, B_w_up, B_w_down)
    return h2
```

```python
import math

import jax
import jax.numpy as jnp
from jax import lax
import jax.experimental.pallas as pl
import jax.experimental.pallas.tpu as pltpu

_H = 32
_EPS = 1e-5
_LANES = 128
_RB = 512
_FIRST_ROWS = 128
_TQ = 512
_KB = 128
_VK = 16
_UNROLL = 2
_SKEW = 1
_AHEAD = 1
_VPU_LAG = 7
_KEY_PARTS = 2
_STAGE_LAG = 5
_SUM_MIN = 2.0 ** -75
_FB = 256
_BF16_ONE_PAIR = 0x3F803F80

_F32 = jnp.float32
_BF16 = jnp.bfloat16


def _layernorm(x):
    mean = jnp.mean(x, axis=-1, keepdims=True)
    xc = x - mean
    var = jnp.mean(xc * xc, axis=-1, keepdims=True)
    return xc * lax.rsqrt(var + _EPS)


def _dot(a, b):
    return jnp.dot(a, b, preferred_element_type=_F32)


def _dot_nt(a, b):
    return lax.dot_general(a, b, (((1,), (1,)), ((), ())), preferred_element_type=_F32)


def _silu(x):
    half = 0.5 * x
    return half * jnp.tanh(half) + half


def _strassen_lhs(a11, a12, a21, a22):
    terms = (a11 + a22, a21 + a22, a11, a22, a11 + a12, a21 - a11, a12 - a22)
    return [t.astype(_BF16) for t in terms]


def _strassen_rhs(b11, b12, b21, b22):
    terms = (b11 + b22, b12 - b22, b21 - b11, b11 + b12, b21 + b22)
    return [t.astype(_BF16) for t in terms]


def _with_plain(sums, b11, b22):
    return [sums[0], b11, sums[1], sums[2], b22, sums[3], sums[4]]


def _strassen_out(m):
    return (m[0] + m[3] - m[4] + m[6], m[2] + m[4], m[1] + m[3], m[0] - m[1] + m[2] + m[5])


def _block_kernel(x_hbm, wqkv_hbm, wo_hbm, wg_hbm, wu_hbm, wd_hbm, out_hbm,
                  x_v, xn_v, wqkv_v, wt_v, wo_v, wg_v, wu_v, wd_v,
                  qt_v, qf_v, k_v, vt_v, ot_v, shift_v, ka0_v, kb0_v, ka1_v, kb1_v, p_v,
                  wgu_v, wds_v, h_v, hn_v, act_v, out_v,
                  x_sems, w_sems, out_sems):
    S, D = x_v.shape
    F = wg_v.shape[1]
    dh = D // _H
    n_rb = S // _RB
    n_qb = S // _TQ
    n_kb = S // _KB
    n_items = _H * n_qb
    q_scale = dh ** -0.5 * math.log2(math.e)

    segs = [(0, _FIRST_ROWS), (_FIRST_ROWS, _RB - _FIRST_ROWS)] + [(r * _RB, _RB) for r in range(1, n_rb)]

    def x_copy(i):
        rows = pl.ds(*segs[i])
        return pltpu.make_async_copy(x_hbm.at[rows], x_v.at[rows], x_sems.at[i])

    wq_copy, wk_copy, wv_copy = [
        pltpu.make_async_copy(wqkv_hbm.at[:, pl.ds(i * D, D)], wqkv_v.at[i],
                              w_sems.at[i]) for i in range(3)]
    wo_copy, wg_copy, wu_copy, wd_copy = [
                   pltpu.make_async_copy(src, dst, w_sems.at[3 + i])
                   for i, (src, dst) in enumerate(
                       [(wo_hbm, wo_v), (wg_hbm, wg_v), (wu_hbm, wu_v), (wd_hbm, wd_v)])]

    def ln1(i):
        rows = pl.ds(*segs[i])
        xn_v[rows, :] = _layernorm(x_v[rows, :].astype(_F32)).astype(_BF16)

    def k_proj(i):
        r0, n = segs[i]
        k = _dot(xn_v[pl.ds(r0, n), :], wqkv_v[1]).astype(_BF16)
        for g in range(D // _LANES):
            k_v[g, pl.ds(r0 // 2, n // 2), :] = pltpu.bitcast(
                k[:, g * _LANES:(g + 1) * _LANES], jnp.int32)

    def q_proj(r):
        qt = (_dot_nt(wt_v[0], xn_v[pl.ds(r * _RB, _RB), :]) * q_scale).astype(_BF16)
        qt_v[r] = qt
        qf = qt.astype(_F32)
        qf_v[r] = qf
        for h in range(_H):
            qh = qf[h * dh:(h + 1) * dh]
            shift_v[r, h:h + 1, :] = jnp.sum(qh * qh, axis=0, keepdims=True)

    def finish_shifts():
        k2 = None
        for r in range(n_rb):
            rows = pl.ds(r * _RB // 2, _RB // 2)
            k = jnp.concatenate([pltpu.bitcast(k_v[g, rows, :], _BF16)
                                 for g in range(D // _LANES)], axis=1).astype(_F32)
            k2 = k * k if k2 is None else jnp.maximum(k2, k * k)
        head_of = (lax.broadcasted_iota(jnp.int32, (_H, D), 1) // dh
                   == lax.broadcasted_iota(jnp.int32, (_H, D), 0))
        k2 = _dot_nt(jnp.where(head_of, 1.0, 0.0).astype(_BF16), k2.astype(_BF16))
        k2 = jnp.max(k2, axis=1, keepdims=True)
        for r in range(n_qb):
            shift_v[r] = jnp.sqrt(shift_v[r] * k2).astype(_BF16).astype(_F32)

    def v_proj(r, d0=0, nd=D):
        rows = pl.ds(r * _RB, _RB)
        vt = _dot_nt(wt_v[1, d0:d0 + nd, :], xn_v[rows, :])
        vt_v[d0:d0 + nd, rows] = vt.astype(_BF16)
        return vt

    hm, hd, hf = _FB // 2, D // 2, F // 2

    def quadrants(w, rows, cols):
        (r0, nr), (c0, nc) = rows, cols
        dr, dc = w.shape[0] // 2, w.shape[1] // 2
        return [w[pl.ds(r0 + i * dr, nr), pl.ds(c0 + j * dc, nc)] for i in (0, 1) for j in (0, 1)]

    n_chunks = hf // _LANES
    slab = 32
    unpaced = lax.broadcasted_iota(jnp.int32, (slab, _LANES), 0) >= pl.program_id(0)

    def stage_weights(c, n, r, tick):
        if n < 2:
            blocks = quadrants((wg_v, wu_v)[n], (r, slab), (c * _LANES, _LANES))
            dst, where = wgu_v, (pl.ds(r, slab), pl.ds((2 * c + n) * _LANES, _LANES))
        else:
            blocks = quadrants(wd_v, (c * _LANES + r, slab), (0, hd))
            dst, where = wds_v, (pl.ds(c * _LANES + r, slab), slice(None))
        reps, tick = blocks[0].shape[1] // _LANES, tick.astype(blocks[0].dtype)
        blocks = [jnp.concatenate(
            [jnp.where(unpaced, t[:, i * _LANES:(i + 1) * _LANES], tick).astype(_F32)
             for i in range(reps)], axis=1) for t in blocks]
        for i, term in enumerate(_strassen_rhs(*blocks)):
            dst[(i,) + where] = term

    def weight_pieces(n):
        return [(c, n, r) for c in range(n_chunks) for r in range(0, hd if n < 2 else _LANES, slab)]

    def stage_along(pieces, share, n_shares, result):
        pieces = pieces[share * len(pieces) // n_shares:(share + 1) * len(pieces) // n_shares]
        for k, piece in enumerate(pieces):
            t0 = (k * (result.shape[0] // slab)) // len(pieces) * slab
            stage_weights(*piece, result[t0:t0 + slab, :_LANES])

    x_copy(0).start()
    wk_copy.start()
    x_copy(1).start()
    x_copy(0).wait()
    wq_copy.start()
    x_copy(2).start()
    ln1(0)
    wk_copy.wait()
    x_copy(1).wait()
    k_proj(0)
    ln1(1)
    k_proj(1)
    wq_copy.wait()
    x_copy(2).wait()
    wv_copy.start()
    for i in range(3, len(segs)):
        x_copy(i).start()
    wt_v[0] = wqkv_v[0].T
    q_proj(0)
    ln1(2)
    k_proj(2)
    q_proj(1)
    wv_copy.wait()
    for i in range(3, len(segs)):
        x_copy(i).wait()
    wg_copy.start()
    wu_copy.start()
    wt_v[1] = wqkv_v[2].T
    v_proj(0)
    for i in range(3, len(segs)):
        ln1(i)
        k_proj(i)
    for r in range(2, n_rb):
        q_proj(r)

    def head_rows(h):
        return pl.ds(pl.multiple_of(h * dh, dh), dh)

    heads_per_vreg = _LANES // dh
    n_sub = _KB // 8
    key_slots = ((ka0_v, kb0_v), (ka1_v, kb1_v))

    n_steps = n_qb * n_kb
    words = _KB // 2

    def head_keys(h, row, n, gate=lambda v: v):
        k = gate(k_v[h // heads_per_vreg, pl.ds(pl.multiple_of(row, 8), n), :])
        return pltpu.roll(k, (_LANES - (h % heads_per_vreg) * dh) % _LANES, 1)

    def stage_keys(h, j, part, slot, gate=lambda v: v):
        ka_v, kb_v = key_slots[slot]
        n = words // _KEY_PARTS
        k = head_keys(h, j * words + part * n, n, gate)
        data_lanes = lax.broadcasted_iota(jnp.int32, k.shape, 1) < dh
        ka_v[j, part * n:(part + 1) * n, :] = jnp.where(data_lanes, k, _BF16_ONE_PAIR)
        kf = head_keys(h, (j + 1) * words - _VK // 2, _VK // 2, gate)
        kf = pltpu.bitcast(kf, _BF16).astype(_F32)
        for d in range(part * dh // _KEY_PARTS, (part + 1) * dh // _KEY_PARTS):
            kb_v[j, d] = jnp.broadcast_to(kf[:, d:d + 1], (_VK, _LANES))

    def check_sums(unsafe, l):
        return jnp.where(jnp.logical_and(l >= _SUM_MIN, l <= 2.0 * S), unsafe, 1)

    def finish_item(h, qb, o, l):
        ot_v[qb, head_rows(h), :] = (o * (1.0 / l)).astype(_BF16)

    def attn_heads(it, carry):
        unsafe, o, l8 = carry
        first_row = lax.broadcasted_iota(jnp.int32, (dh, _TQ), 0) == 0
        always = jnp.full((8, _LANES), it, jnp.int32) < _H
        ticks, pv_ticks = [], []

        def gated(v, src, source=ticks, half=0, col=0):
            if src < 0:
                return v
            tick = source[src][half * 8:half * 8 + 8, col * _LANES:(col + 1) * _LANES]
            tick = pltpu.bitcast(tick, v.dtype)
            return jnp.concatenate(
                [jnp.concatenate([jnp.where(always, v[r:r + 8, c:c + _LANES], tick)
                                  for c in range(0, v.shape[1], _LANES)], axis=1)
                 for r in range(0, v.shape[0], 8)], axis=0)

        def decode(t):
            u, t = divmod(t, n_steps)
            return u, t // n_kb, t % n_kb

        queries = {}

        def item_queries(u, qb):
            if (u, qb) not in queries:
                h = it * _UNROLL + u
                qt = qt_v[qb, head_rows(h), :]
                shift = shift_v[qb, pl.ds(h, 1), :]
                q_aug = jnp.concatenate(
                    [qt, jnp.where(first_row, -shift, 0.0).astype(_BF16)], axis=0)
                queries[u, qb] = (
                    q_aug, jnp.broadcast_to(-shift, (8, _TQ)),
                    [jnp.broadcast_to(qf_v[qb, pl.ds(h * dh + d, 1), :], (8, _TQ)) for d in range(dh)])
            return queries[u, qb]

        stream, begin = [], []
        for t in range(_UNROLL * n_steps):
            begin.append(len(stream))
            stream += [(t, g) for g in reversed(range((_KB - _VK) // 16))]
        begin.append(len(stream))
        scores = {}
        pending = [p_v[i] for i in range(_SKEW)]
        sums = [jnp.sum(l8, axis=0, keepdims=True)]

        def pv_step(t, o):
            u2, t2 = divmod(t - _SKEW, n_steps)
            qb2, j2 = divmod(t2, n_kb)
            h2 = jnp.maximum(it * _UNROLL + u2, 0)
            pv = _dot(vt_v[head_rows(h2), pl.ds(j2 * _KB, _KB)], pending[t])
            pv_ticks.append(pv)
            o = pv if j2 == 0 else o + pv
            if j2 == n_kb - 1:
                finish_item(h2, qb2, o, sums[(t - _SKEW) // n_kb + 1])
            return o

        for t in range(_UNROLL * n_steps):
            u, qb, j = decode(t)
            h = it * _UNROLL + u
            todo = stream[len(ticks):begin[t + 1] + _AHEAD]
            for item in sorted({t2 // n_kb for t2, _ in todo}):
                grp = [(t2, g) for t2, g in todo if t2 // n_kb == item]
                u1, qb1, _ = decode(item * n_kb)
                k = jnp.concatenate(
                    [key_slots[u1 % 2][0][t2 % n_kb, g * 8:(g + 1) * 8, :] for t2, g in grp], axis=0)
                s = _dot(pltpu.bitcast(k, _BF16)[:, :2 * dh], item_queries(u1, qb1)[0])
                for n, key in enumerate(grp):
                    scores[key] = s[n * 16:(n + 1) * 16]
                    ticks.append(s[n * 16:(n + 1) * 16])
            parts = [scores.pop((t, g)) for g in range(begin[t + 1] - begin[t])]
            n8 = _VK // 8
            pace = [(g - _VPU_LAG, ticks) for g in range(begin[t], begin[t + 1])]
            pace.insert(_AHEAD + _VPU_LAG - len(pace), (t - 2, pv_ticks))
            acc = [item_queries(u, qb)[1]] * n8
            for n in range(dh * n8):
                d, i = divmod(n, n8)
                kb = gated(key_slots[u % 2][1][j, d, i * 8:(i + 1) * 8, :],
                           *pace[(n * len(pace)) // (dh * n8)], half=n // 2 % 2, col=_TQ // _LANES - 1)
                if i == 0:
                    q_row = item_queries(u, qb)[2][d]
                acc[i] = acc[i] + jnp.concatenate([kb] * (_TQ // _LANES), axis=1) * q_row
            p = jnp.exp2(jnp.concatenate(parts + acc, axis=0))
            pending.append(p.astype(_BF16))
            rows = [p[r * 8:(r + 1) * 8] for r in reversed(range(n_sub))]
            rows = rows[2:4] + rows[:2] + rows[4:]
            lj = sum(rows[1:], rows[0])
            l8 = lj if j == 0 else l8 + lj
            if j == n_kb - 1:
                sums.append(jnp.sum(l8, axis=0, keepdims=True))

            o = pv_step(t, o)

            h_next = jnp.minimum(h + 1, _H - 1)
            part, rem = divmod(t % n_steps, n_qb // _KEY_PARTS)
            if rem == 1:
                stage_keys(h_next, part // _KEY_PARTS, part % _KEY_PARTS, (u + 1) % 2,
                           lambda v: gated(v, begin[t] - _STAGE_LAG))
        for i in range(_SKEW):
            p_v[i] = pending[_UNROLL * n_steps + i]
        for l in sums[:-1]:
            unsafe = check_sums(unsafe, l)
        return unsafe, o, l8

    for j in range(n_kb):
        for part in range(_KEY_PARTS):
            stage_keys(0, j, part, 0)
    p_v[...] = jnp.zeros(p_v.shape, _BF16)

    wg_copy.wait()
    wu_copy.wait()
    wo_copy.start()
    wd_copy.start()
    finish_shifts()
    pieces = weight_pieces(0) + weight_pieces(1)
    dots = [(r, d0) for r in range(1, n_rb) for d0 in range(0, D, D // 4)]
    for k, (r, d0) in enumerate(dots):
        stage_along(pieces, k, len(dots), v_proj(r, d0, D // 4))

    unsafe, o, l8 = lax.fori_loop(
        0, _H // _UNROLL, attn_heads,
        (jnp.zeros((1, _TQ), jnp.int32), jnp.zeros((dh, _TQ), _F32), jnp.ones((8, _TQ), _F32)))
    l = jnp.sum(l8, axis=0, keepdims=True)
    for i in range(_SKEW):
        o = o + _dot(vt_v[head_rows(_H - 1), pl.ds((n_kb - _SKEW + i) * _KB, _KB)],
                     p_v[i])
    finish_item(_H - 1, n_qb - 1, o, l)

    n_unsafe = jnp.sum(check_sums(unsafe, l))

    @pl.when(n_unsafe > 0)
    def _():
        def true_max_item(item, _):
            h, qb = item // n_qb, item % n_qb
            qt = qt_v[qb, head_rows(h), :]

            def block(j, state):
                m, l, acc = state
                keys = pl.ds(pl.multiple_of(j * _KB, _KB), _KB)
                s = _dot(pltpu.bitcast(head_keys(h, j * words, words), _BF16)[:, :dh], qt)
                m_new = jnp.maximum(m, jnp.max(s, axis=0, keepdims=True))
                p = jnp.exp2(s - m_new)
                alpha = jnp.exp2(m - m_new)
                l = alpha * l + jnp.sum(p, axis=0, keepdims=True)
                return m_new, l, alpha * acc + _dot(vt_v[head_rows(h), keys], p.astype(_BF16))

            init = (jnp.full((1, _TQ), -jnp.inf, _F32), jnp.zeros((1, _TQ), _F32),
                    jnp.zeros((dh, _TQ), _F32))
            _, l, acc = lax.fori_loop(0, n_kb, block, init)
            finish_item(h, qb, acc, l)

        lax.fori_loop(0, n_items, true_max_item, None)

    wo_copy.wait()
    wd_copy.wait()

    for r in range(S // _FB):
        rows = pl.ds(r * _FB, _FB)
        attn = _dot(ot_v[r * _FB // _TQ, :, pl.ds(r * _FB % _TQ, _FB)].T, wo_v[...])
        stage_along(weight_pieces(2), r, S // _FB - 1, attn)
        h = x_v[rows, :].astype(_F32) + attn
        h_v[rows, :] = h
        hn = _layernorm(h)
        terms = _strassen_lhs(hn[:hm, :hd], hn[:hm, hd:], hn[hm:, :hd], hn[hm:, hd:])
        for i, term in enumerate(terms):
            hn_v[r, i] = term

    def out_copy(r):
        rows = pl.ds(pl.multiple_of(r * _FB, _FB), _FB)
        return pltpu.make_async_copy(out_v.at[rows], out_hbm.at[rows], out_sems.at[r])

    def ffn_block(r, _):
        rows = pl.ds(pl.multiple_of(r * _FB, _FB), _FB)
        for c in range(n_chunks):
            cols = pl.ds(2 * c * _LANES, 2 * _LANES)
            g, u = [quadrants(w, (0, hd), (c * _LANES, _LANES)) for w in (wg_v, wu_v)]
            rhs = _with_plain([wgu_v[i, :, cols] for i in range(5)],
                              *[jnp.concatenate([g[i], u[i]], axis=1) for i in (0, 3)])
            gu = _strassen_out([_dot(hn_v[r, i], rhs[i]) for i in range(7)])
            act = [_silu(t[:, :_LANES]) * t[:, _LANES:] for t in gu]
            for i, term in enumerate(_strassen_lhs(*act)):
                act_v[i, :, pl.ds(c * _LANES, _LANES)] = term
        rhs = _with_plain([wds_v[i] for i in range(5)], wd_v[:hf, :hd], wd_v[hf:, hd:])
        y = _strassen_out([_dot(act_v[i], rhs[i]) for i in range(7)])
        y = jnp.concatenate([jnp.concatenate(y[:2], axis=1), jnp.concatenate(y[2:], axis=1)], axis=0)
        out_v[rows, :] = (h_v[rows, :] + y).astype(out_v.dtype)
        out_copy(r).start()

    lax.fori_loop(0, S // _FB, ffn_block, None)
    for r in range(S // _FB):
        out_copy(r).wait()


@jax.jit
def pallas_sequential_preLN__softmax_full_mha__swiglu_ffn__prompt_kernel(
    A_x: jax.Array,
    A_wqkv: jax.Array,
    A_wo: jax.Array,
    B_x: jax.Array,
    B_w_gate: jax.Array,
    B_w_up: jax.Array,
    B_w_down: jax.Array,
):
    del B_x
    B, S, D = A_x.shape
    F = B_w_gate.shape[1]
    assert B == 1 and _RB == _TQ and S % _RB == 0 and F % (2 * _LANES) == 0
    n_rb = S // _RB
    vmem = pltpu.VMEM
    key_slot = [vmem((S // _KB, _KB // 2, _LANES), jnp.int32),
                vmem((S // _KB, D // _H, _VK, _LANES), _F32)]
    out = pl.pallas_call(
        _block_kernel,
        out_shape=jax.ShapeDtypeStruct((S, D), A_x.dtype),
        grid=(1,),
        in_specs=[pl.BlockSpec(memory_space=pl.ANY)] * 6,
        out_specs=pl.BlockSpec(memory_space=pl.ANY),
        scratch_shapes=[
            vmem((S, D), A_x.dtype),
            vmem((S, D), _BF16),
            vmem((3, D, D), A_wqkv.dtype),
            vmem((2, D, D), A_wqkv.dtype),
            vmem((D, D), A_wo.dtype),
            vmem((D, F), B_w_gate.dtype),
            vmem((D, F), B_w_up.dtype),
            vmem((F, D), B_w_down.dtype),
            vmem((S // _TQ, D, _TQ), _BF16),
            vmem((S // _TQ, D, _TQ), _F32),
            vmem((D // _LANES, S // 2, _LANES), jnp.int32),
            vmem((D, S), _BF16),
            vmem((S // _TQ, D, _TQ), _BF16),
            vmem((S // _TQ, _H, _TQ), _F32),
            *key_slot, *key_slot,
            vmem((_SKEW, _KB, _TQ), _BF16),
            vmem((5, D // 2, F), _BF16),
            vmem((5, F // 2, D // 2), _BF16),
            vmem((S, D), _F32),
            vmem((S // _FB, 7, _FB // 2, D // 2), _BF16),
            vmem((7, _FB // 2, F // 2), _BF16),
            vmem((S, D), A_x.dtype),
            pltpu.SemaphoreType.DMA((n_rb + 1,)),
            pltpu.SemaphoreType.DMA((7,)),
            pltpu.SemaphoreType.DMA((S // _FB,)),
        ],
        compiler_params=pltpu.CompilerParams(vmem_limit_bytes=100 * 1024 * 1024),
    )(A_x.reshape(S, D), A_wqkv, A_wo, B_w_gate, B_w_up, B_w_down)
    return out.reshape(B, S, D)
```
